```python
import os as _os
_os.environ.setdefault("JAX_PLATFORMS", "cpu")
import jax
import jax.numpy as jnp

def _softmax(x, axis=-1):
    return jax.nn.softmax(x, axis=axis)
def _gelu(x):
    return jax.nn.gelu(x, approximate=True)
def _silu(x):
    return jax.nn.silu(x)
def _sigmoid(x):
    return jax.nn.sigmoid(x)
def _layernorm(x, axis=-1, eps=1e-5):
    m = jnp.mean(x, axis=axis, keepdims=True)
    v = jnp.var(x, axis=axis, keepdims=True)
    return (x - m) / jnp.sqrt(v + eps)
def _scatter_add(tgt, idx, src, axis=0):
    return tgt.at[idx].add(src)
def _segment_sum(src, seg, n):
    return jax.ops.segment_sum(src, seg, n)
class _Rng:
    def __init__(self, key):
        self._k = key
    def _next(self):
        self._k, sub = jax.random.split(self._k)
        return sub
    def normal(self, shape):
        return jax.random.normal(self._next(), shape, dtype=jnp.bfloat16)
    def randint(self, lo, hi, shape):
        return jax.random.randint(self._next(), shape, lo, hi, dtype=jnp.int32)
    def uniform(self, shape, lo=0.0, hi=1.0):
        return jax.random.uniform(self._next(), shape, jnp.bfloat16, lo, hi)
    def permutation(self, n):
        return jax.random.permutation(self._next(), n)


kernel_name = 'parallel_sum__linear_kernel_hedgehog__dense_activation_gelu__prompt'

def setup_inputs():
    _rng = _Rng(jax.random.key(int.from_bytes(__import__("os").urandom(4), "little")))
    _w = (lambda a: (lambda t: t.astype(jnp.bfloat16) if jnp.issubdtype(t.dtype, jnp.floating) else t)(jnp.asarray(a)))
    def _A_setup():
        B, S, D, H = 1, 2048, 448, 16
        Dh = D // H
        return {
            "x": _w((lambda *s: _rng.normal(s) * 0.05)(B, S, D)),
            "wqkv": _w((lambda *s: _rng.normal(s) * 0.2)(D, 3 * D)),
            "w_phi": _w((lambda *s: _rng.normal(s) * 0.2)(H, Dh, Dh) * (Dh ** -0.5)),
            "wo": _w((lambda *s: _rng.normal(s) * 0.05)(D, D)),
        }
    _A_in = _A_setup()

    def _B_setup():
        B, S, D, F = 1, 2048, 448, 1792
        return {
            "x": _w((lambda *s: _rng.normal(s) * 0.05)(B, S, D)),
            "w1": _w((lambda *s: _rng.normal(s) * 0.2)(D, F) * (D ** -0.5)),
            "b1": _w((lambda *s: _rng.normal(s) * 0.2)(F) * 0.01),
            "w2": _w((lambda *s: _rng.normal(s) * 0.2)(F, D) * (F ** -0.5)),
            "b2": _w((lambda *s: _rng.normal(s) * 0.05)(D) * 0.01),
        }
    _B_in = _B_setup()

    return {
        "A_x": _A_in["x"],
        "A_wqkv": _A_in["wqkv"],
        "A_w_phi": _A_in["w_phi"],
        "A_wo": _A_in["wo"],
        "B_x": _B_in["x"],
        "B_w1": _B_in["w1"],
        "B_b1": _B_in["b1"],
        "B_w2": _B_in["w2"],
        "B_b2": _B_in["b2"],
    }

def reference(A_x, A_wqkv, A_w_phi, A_wo, B_x, B_w1, B_b1, B_w2, B_b2):
    def _A_ref(x, wqkv, w_phi, wo):
        B, S, D = x.shape
        H = 16; Dh = D // H
        qkv = (lambda x, *d: x.transpose(*d))((x @ wqkv).reshape(B, S, 3, H, Dh), 2, 0, 3, 1, 4)
        q, k, v = qkv[0], qkv[1], qkv[2]
        pq = jnp.einsum("bhsd,hdf->bhsf", q, w_phi)
        pk = jnp.einsum("bhsd,hdf->bhsf", k, w_phi)
        phi_q = jnp.concatenate([_softmax(pq, axis=-1), _softmax(-pq, axis=-1)], axis=-1)
        phi_k = jnp.concatenate([_softmax(pk, axis=-1), _softmax(-pk, axis=-1)], axis=-1)
        kv = jnp.einsum("bhsf,bhsd->bhfd", phi_k, v)
        z  = jnp.einsum("bhsf->bhf", phi_k)
        num = jnp.einsum("bhqf,bhfd->bhqd", phi_q, kv)
        den = jnp.einsum("bhqf,bhf->bhq", phi_q, z)[..., None] + 1e-6
        o = num / den
        return (lambda x, *d: x.transpose(*d))(o, 0, 2, 1, 3).reshape(B, S, D) @ wo

    def _B_ref(x, w1, b1, w2, b2):
        h = jnp.einsum("bsd,df->bsf", x, w1) + b1
        h = _gelu(h)
        return jnp.einsum("bsf,fd->bsd", h, w2) + b2

    x = A_x
    xn = _layernorm(x, axis=-1)
    return x + _A_ref(xn, A_wqkv, A_w_phi, A_wo) + _B_ref(xn, B_w1, B_b1, B_w2, B_b2)
```

```python
import functools
import jax
import jax.numpy as jnp
from jax import lax
import jax.experimental.pallas as pl
import jax.experimental.pallas.tpu as pltpu

S, D, H, DH, F = 2048, 448, 16, 28, 1792
DP = 512
G = 8
GR = 2 * DH
TS = 512
T = S // TS
EPS = 1e-5
VAR = 'F'
CW = 256
CPT = TS // CW
NC = S // CW
NT = (((1,), (1,)), ((), ()))
f32 = jnp.float32
bf16 = jnp.bfloat16


def _dot(a, b):
    return jnp.dot(a, b, preferred_element_type=f32)


def _dot_nt(a, b):
    return lax.dot_general(a, b, NT, preferred_element_type=f32)


def _feature_map(pT):
    n = pT.shape[-1]
    p = pT.reshape(G, 7, 8, n)

    def allred(x, op):
        x = op(x, pltpu.roll(x, 2, 1))
        return op(x, pltpu.roll(x, 4, 1))

    mx = allred(jnp.max(p, axis=1), jnp.maximum)
    mn = allred(jnp.min(p, axis=1), jnp.minimum)
    ep = jnp.exp(p - mx[:, None])
    en = jnp.exp(mn[:, None] - p)
    sp = allred(jnp.sum(ep, axis=1), jnp.add)
    sn = allred(jnp.sum(en, axis=1), jnp.add)
    ep = ep * (1.0 / sp)[:, None]
    en = en * (1.0 / sn)[:, None]
    phi = jnp.concatenate([ep, en], axis=1)
    return phi.reshape(G, 2 * GR, n).astype(bf16)


def _tiles(base):
    out = []
    for t in range(base // 128, (base + D - 1) // 128 + 1):
        g_lo = max((128 * t - base) // GR, 0)
        g_hi = min((128 * t + 127 - base) // GR, G - 1)
        out.append((t, g_lo, g_hi))
    return out


def _bdt_blocks(a_scr, base):
    blocks = []
    for t, g_lo, g_hi in _tiles(base):
        m = (g_hi - g_lo + 1) * GR
        r = lax.broadcasted_iota(jnp.int32, (m, 128), 0) + g_lo * GR
        c = lax.broadcasted_iota(jnp.int32, (m, 128), 1)
        g = (r * 1171) >> 16
        fr = (r - g * GR) >> 1
        selT = jnp.where(fr == c, 1.0, 0.0).astype(bf16)
        a = a_scr[128 * t:128 * (t + 1), :].astype(bf16)
        full = _dot_nt(selT, a)
        lo = (2 * g + (r & 1)) * DH + (base - 128 * t)
        blocks.append(jnp.where((c >= lo) & (c < lo + DH), full, 0.0).astype(bf16))
    return blocks


def _folded_weight(blocks, wqkv_scr, base):
    pieces = [None] * G
    for bdt, (t, g_lo, g_hi) in zip(blocks, _tiles(base)):
        part = _dot_nt(bdt, wqkv_scr[:, 128 * t:128 * (t + 1)])
        for gg in range(g_lo, g_hi + 1):
            p = part[(gg - g_lo) * GR:(gg - g_lo + 1) * GR]
            pieces[gg] = p if pieces[gg] is None else pieces[gg] + p
    return jnp.concatenate(pieces, axis=0)


def _schedule():
    out = []
    LA = CPT
    def extras(c):
        e = []
        if c == 1 * CPT: e.append(('wq', 0))
        if CPT == 1:
            if c == 2: e += [('w1t', (1, 0))]
        else:
            if c == 2 * CPT: e.append(('w1t', (2, 0)))
            if c == 2 * CPT + CPT // 2: e.append(('w1t', (2, 1)))
        if c == 3 * CPT: e.append(('wot', 0))
        return e
    def waits(c):
        w = []
        if c % CPT == 0:
            t = c // CPT
            if t + 1 < T: w.append(('wx', t + 1))
            if t == 0: w.append(('start2', 0))
            if t == 1: w.append(('wwq', 0))
            if t == 2: w.append(('ww1', 0))
            if t == 3: w.append(('wwo', 0))
        return w
    if VAR in ('A', 'B', 'C'):
        out.append(('pk', 0))
    for c in range(NC):
        out += waits(c)
        ln = [('ln', c + LA)] if c + LA < NC else []
        pkn = [('pk', c + 1)] if c + 1 < NC else []
        if VAR == 'A':
            out += pkn + [('phi', c), ('v', c)] + ln + extras(c) + [('kv', c)]
        elif VAR == 'B':
            out += pkn + [('phi', c), ('v', c)] + ln + extras(c) + ([('kv', c - 1)] if c > 0 else [])
        elif VAR == 'C':
            out += ln + pkn + [('phi', c), ('v', c)] + extras(c) + ([('kv', c - 1)] if c > 0 else [])
        elif VAR == 'D':
            out += [('pkphi', c)] + ln + [('v', c)] + extras(c) + [('kv', c)]
        elif VAR == 'E':
            out += [('pkphi', c)] + ln + [('v', c)] + extras(c) + ([('kv', c - 1)] if c > 0 else [])
        elif VAR == 'F':
            out += [('v', c)] + ln + [('pkphi', c)] + extras(c) + ([('kv', c - 1)] if c > 0 else [])
        elif VAR == 'G':
            out += [('pkphi', c), ('v', c)] + ln + extras(c) + ([('kv', c - 1)] if c > 0 else [])
    if VAR in ('B', 'C', 'E', 'F', 'G'):
        out.append(('kv', NC - 1))
    return out


def _kernel(x_hbm, wqkv_hbm, wphi_ref, b1_ref, b2_ref, wo_hbm, w1_hbm, w2T_hbm, o_ref,
            x_scr, xn_scr, wqkv_scr, wk_scr, wv_scr, wq_scr, w1raw, w1T, w2T, woraw, woT,
            p_scr, a_scr, kvT, pk_scr, phi_scr, va_scr, kv_acc, sems):
    i = pl.program_id(0)

    def x_copy(t):
        return pltpu.make_async_copy(x_hbm.at[:, pl.ds(t * TS, TS)], x_scr.at[:, pl.ds(t * TS, TS)], sems.at[t])

    def wqkv_copy(k):
        lo, hi = [(384, 896), (896, 1344), (0, 384)][k]
        return pltpu.make_async_copy(wqkv_hbm.at[:, pl.ds(lo, hi - lo)], wqkv_scr.at[:, pl.ds(lo, hi - lo)],
                                     sems.at[T + k])

    def w1_copy():
        return pltpu.make_async_copy(w1_hbm, w1raw.at[pl.ds(0, D), :], sems.at[T + 3])

    def wo_copy():
        return pltpu.make_async_copy(wo_hbm, woraw.at[pl.ds(0, D), :], sems.at[T + 4])

    def w2_copy():
        return pltpu.make_async_copy(w2T_hbm, w2T, sems.at[T + 5])

    def layernorm(c):
        x = x_scr[:, c * CW:(c + 1) * CW].astype(f32)
        m = jnp.mean(x, axis=0, keepdims=True)
        xc = x - m
        var = jnp.mean(xc * xc, axis=0, keepdims=True)
        xn = xc * lax.rsqrt(var + EPS)
        rr = lax.broadcasted_iota(jnp.int32, (DP - D, CW), 0)
        xa = jnp.concatenate([xn, jnp.where(rr == 0, 1.0, 0.0)], axis=0).astype(bf16)
        xn_scr[c // CPT, :, (c % CPT) * CW:(c % CPT + 1) * CW] = xa

    def xa_chunk(c):
        return xn_scr[c // CPT, :, (c % CPT) * CW:(c % CPT + 1) * CW]

    def pk_chunk(c):
        pk_scr[c % 2] = _dot(wk_scr[...], xa_chunk(c))

    def phi_chunk(c):
        phi_scr[c % 2] = _feature_map(pk_scr[c % 2])

    def v_chunk(c):
        vT = _dot(wv_scr[...], xa_chunk(c)).reshape(G, GR, CW)
        ones = jnp.ones((G, 8, CW), f32)
        va_scr[c % 2] = jnp.concatenate([vT, ones], axis=1).astype(bf16)

    def kv_chunk(c):
        for g in range(G):
            new = _dot_nt(va_scr[c % 2, g], phi_scr[c % 2, g])
            if c == 0:
                kv_acc[g] = new
            else:
                kv_acc[g] += new

    @pl.when(i == 0)
    def _():
        x_copy(0).start()
        wqkv_copy(0).start()
        wqkv_copy(1).start()
        x_copy(1).start()
        p_scr[...] = jnp.zeros(p_scr.shape, f32)
        p_scr[:, 0:DH] = wphi_ref[...].reshape(D, DH).astype(f32)
        for h in range(H):
            blk = p_scr[pl.ds(h, DH, stride=H), :]
            a_scr[DH * h:DH * (h + 1), :] = blk
            a_scr[D + DH * h:D + DH * (h + 1), :] = blk
        zpad = jnp.zeros((D, DP - D), bf16)
        wk_scr[:, D:DP] = zpad
        wv_scr[:, D:DP] = zpad
        wq_scr[:, D:DP] = zpad
        bdt_k = _bdt_blocks(a_scr, D)
        x_copy(0).wait()
        for c in range(CPT):
            layernorm(c)
        wqkv_copy(0).wait()
        wqkv_copy(1).wait()
        x_copy(2).start()
        wqkv_copy(2).start()
        x_copy(3).start()
        w1_copy().start()
        wk_scr[:, 0:D] = _folded_weight(bdt_k, wqkv_scr, D).astype(bf16)
        wv_scr[:, 0:D] = wqkv_scr[:, 896:1344].T
        for item in _schedule():
            kind, c = item
            if kind == 'wx':
                x_copy(c).wait()
            elif kind == 'start2':
                wo_copy().start()
                w2_copy().start()
            elif kind == 'wwq':
                wqkv_copy(2).wait()
            elif kind == 'ww1':
                w1_copy().wait()
            elif kind == 'wwo':
                wo_copy().wait()
            elif kind == 'pk':
                pk_chunk(c)
            elif kind == 'phi':
                phi_chunk(c)
            elif kind == 'pkphi':
                phi_scr[c % 2] = _feature_map(_dot(wk_scr[...], xa_chunk(c)))
            elif kind == 'v':
                v_chunk(c)
            elif kind == 'ln':
                layernorm(c)
            elif kind == 'kv':
                kv_chunk(c)
            elif kind == 'wq':
                wq_scr[:, 0:D] = _folded_weight(_bdt_blocks(a_scr, 0), wqkv_scr, 0).astype(bf16)
            elif kind == 'w1t':
                n, k = c
                if k == 0:
                    rr = lax.broadcasted_iota(jnp.int32, (DP - D, F), 0)
                    w1raw[D:DP, :] = jnp.where(rr == 0, b1_ref[...].astype(f32).reshape(1, F), 0.0).astype(bf16)
                hf = F // n
                w1T[k * hf:(k + 1) * hf, :] = w1raw[:, k * hf:(k + 1) * hf].T
            elif kind == 'wot':
                rr = lax.broadcasted_iota(jnp.int32, (DP - D, D), 0)
                woraw[D:DP, :] = jnp.where(rr == 0, b2_ref[...].astype(f32).reshape(1, D), 0.0).astype(bf16)
                woT[...] = woraw[...].T
        r = lax.broadcasted_iota(jnp.int32, (64, 2 * GR), 0)
        c = lax.broadcasted_iota(jnp.int32, (64, 2 * GR), 1)
        hr = jnp.where((r >= DH) & (r < GR) | (r >= 60), 1, 0)
        mask = hr == (c & 1)
        for g in range(G):
            kvT[g] = jnp.where(mask, kv_acc[g], 0.0).astype(bf16)
        w2_copy().wait()

    @pl.when(i > 0)
    def _():
        t = i - 1
        xa = xn_scr[t]
        phi = _feature_map(_dot(wq_scr[...], xa))
        sub = lax.broadcasted_iota(jnp.int32, (8, TS), 0)
        os = []
        for g in range(G):
            nd = _dot(kvT[g], phi[g])
            rd = 1.0 / (nd[GR:64] + 1e-6)
            rr = pltpu.roll(rd, 4, 0)
            r0 = jnp.where(sub < 4, rd, rr)
            r1 = jnp.where(sub < 4, rr, rd)
            scale = jnp.concatenate([r0, r0, r0, rd, r1, r1, r1], axis=0)
            os.append(nd[0:GR] * scale)
        rr = lax.broadcasted_iota(jnp.int32, (DP - D, TS), 0)
        os.append(jnp.where(rr == 0, 1.0, 0.0))
        oT = jnp.concatenate(os, axis=0).astype(bf16)
        hT = _dot(w1T[...], xa)
        c0 = 0.7978845608028654
        u = hT * (c0 + (c0 * 0.044715) * (hT * hT))
        gT = ((0.5 * hT) * (1.0 + jnp.tanh(u))).astype(bf16)
        outT = _dot(woT[...], oT) + _dot(w2T[...], gT)
        col0 = pl.multiple_of(t * TS, TS)
        o_ref[...] = (x_scr[:, pl.ds(col0, TS)].astype(f32) + outT).astype(o_ref.dtype)


@jax.jit
def pallas_parallel_sum__linear_kernel_hedgehog__dense_activation_gelu__prompt_kernel(
        A_x, A_wqkv, A_w_phi, A_wo, B_x, B_w1, B_b1, B_w2, B_b2):
    del B_x
    xT = A_x.reshape(S, D).T
    full = lambda shape: pl.BlockSpec(shape, lambda i: (0,) * len(shape))
    hbm = pl.BlockSpec(memory_space=pl.ANY)
    outT = pl.pallas_call(
        _kernel,
        grid=(T + 1,),
        in_specs=[hbm, hbm, full((DH, H, DH)), full((F,)), full((D,)), hbm, hbm, hbm],
        out_specs=pl.BlockSpec((D, TS), lambda i: (0, jnp.maximum(i - 1, 0))),
        out_shape=jax.ShapeDtypeStruct((D, S), bf16),
        scratch_shapes=[
            pltpu.VMEM((D, S), bf16),
            pltpu.VMEM((T, DP, TS), bf16),
            pltpu.VMEM((D, 3 * D), bf16),
            pltpu.VMEM((D, DP), bf16),
            pltpu.VMEM((D, DP), bf16),
            pltpu.VMEM((D, DP), bf16),
            pltpu.VMEM((DP, F), bf16),
            pltpu.VMEM((F, DP), bf16),
            pltpu.VMEM((D, F), bf16),
            pltpu.VMEM((DP, D), bf16),
            pltpu.VMEM((D, DP), bf16),
            pltpu.VMEM((D, 128), f32),
            pltpu.VMEM((2 * D, 128), f32),
            pltpu.VMEM((G, 64, 2 * GR), bf16),
            pltpu.VMEM((2, D, CW), f32),
            pltpu.VMEM((2, G, 2 * GR, CW), bf16),
            pltpu.VMEM((2, G, 64, CW), bf16),
            pltpu.VMEM((G, 64, 2 * GR), f32),
            pltpu.SemaphoreType.DMA((T + 6,)),
        ],
        compiler_params=pltpu.CompilerParams(
            dimension_semantics=("arbitrary",),
            vmem_limit_bytes=100 * 1024 * 1024,
        ),
    )(xT, A_wqkv, A_w_phi.transpose(1, 0, 2), B_b1, B_b2, A_wo, B_w1, B_w2.T)
    return outT.T.reshape(1, S, D)
```

```python
import jax
import jax.numpy as jnp
from jax import lax
import jax.experimental.pallas as pl
import jax.experimental.pallas.tpu as pltpu

S, D, H, DH, F = 2048, 448, 16, 28, 1792
DP = 512
G = 8
GR = 2 * DH
TS = 512
T = S // TS
UN = 2
CW = 256
NC = S // CW
W1_CHUNK = 6
EPS = 1e-5
LOG2E = 1.4426950408889634
XP = ((0, 256), (256, 768), (768, 2048))
WP = ((384, 896), (896, 1344), (0, 384))
OP = ((0, 384), (384, 512))
NT = (((1,), (1,)), ((), ()))
f32 = jnp.float32
bf16 = jnp.bfloat16
u32 = jnp.uint32


def _pk(x):
    return pltpu.bitcast(x, u32)


def _up(x):
    return pltpu.bitcast(x, bf16)


def _dot(a, b):
    return jnp.dot(a, b, preferred_element_type=f32)


def _dot_nt(a, b):
    return lax.dot_general(a, b, NT, preferred_element_type=f32)


def _feature_map(pT):
    n = pT.shape[-1]
    p = pT.reshape(G, 7, 8, n)

    def allred(x, op):
        x = op(x, pltpu.roll(x, 2, 1))
        return op(x, pltpu.roll(x, 4, 1))

    mx = allred(jnp.max(p, axis=1), jnp.maximum)
    mn = allred(jnp.min(p, axis=1), jnp.minimum)
    ep = jnp.exp2(p - mx[:, None])
    en = jnp.exp2(mn[:, None] - p)
    sp = allred(jnp.sum(ep, axis=1), jnp.add)
    sn = allred(jnp.sum(en, axis=1), jnp.add)
    ep = ep * (1.0 / sp)[:, None]
    en = en * (1.0 / sn)[:, None]
    phi = jnp.concatenate([ep, en], axis=1)
    return phi.reshape(G, 2 * GR, n).astype(bf16)


def _tiles(base):
    out = []
    for t in range(base // 128, (base + D - 1) // 128 + 1):
        g_lo = max((128 * t - base) // GR, 0)
        g_hi = min((128 * t + 127 - base) // GR, G - 1)
        out.append((t, g_lo, g_hi))
    return out


def _bdt_blocks(a_scr, base):
    blocks = []
    for t, g_lo, g_hi in _tiles(base):
        m = (g_hi - g_lo + 1) * GR
        r = lax.broadcasted_iota(jnp.int32, (m, 128), 0) + g_lo * GR
        c = lax.broadcasted_iota(jnp.int32, (m, 128), 1)
        g = (r * 1171) >> 16
        fr = (r - g * GR) >> 1
        selT = jnp.where(fr == c, 1.0, 0.0).astype(bf16)[:, :DH]
        st = 128 * t - base + 64
        a = a_scr[st:st + 128, :].astype(bf16)
        full = _dot_nt(selT, a)
        lo = (2 * g + (r & 1)) * DH + (base - 128 * t)
        blocks.append(jnp.where((c >= lo) & (c < lo + DH), full, 0.0).astype(bf16))
    return blocks


def _folded_weight(blocks, wqkv_scr, base):
    pieces = [None] * G
    for bdt, (t, g_lo, g_hi) in zip(blocks, _tiles(base)):
        part = _dot_nt(bdt, wqkv_scr[:, 128 * t:128 * (t + 1)])
        for gg in range(g_lo, g_hi + 1):
            p = part[(gg - g_lo) * GR:(gg - g_lo + 1) * GR]
            pieces[gg] = p if pieces[gg] is None else pieces[gg] + p
    return (jnp.concatenate(pieces, axis=0) * LOG2E).astype(bf16)


def _kernel(x_hbm, wqkv_hbm, wphi_hbm, b1_hbm, b2_hbm, wo_hbm, w1_hbm, w2T_hbm, o_hbm,
            x_scr, xn_scr, wqkv_scr, wk_scr, wv_scr, wq_scr, w1raw, w1T, w2T, woraw, woT,
            wphi_scr, b1_scr, b2_scr, p_scr, a_scr, kvT, phi_scr, va_scr, kv_acc, o_scr, sems, osems):
    i = pl.program_id(0)

    def x_copy(k):
        lo, hi = XP[k]
        return pltpu.make_async_copy(x_hbm.at[:, pl.ds(lo, hi - lo)], x_scr.at[:, pl.ds(lo, hi - lo)],
                                     sems.at[k])

    def wqkv_copy(k):
        lo, hi = WP[k]
        return pltpu.make_async_copy(wqkv_hbm.at[:, pl.ds(lo, hi - lo)], wqkv_scr.at[:, pl.ds(lo, hi - lo)],
                                     sems.at[3 + k])

    def w1_copy():
        return pltpu.make_async_copy(w1_hbm, w1raw.at[pl.ds(0, D), :], sems.at[6])

    def wo_copy():
        return pltpu.make_async_copy(wo_hbm, woraw.at[pl.ds(0, D), :], sems.at[7])

    def w2_copy():
        return pltpu.make_async_copy(w2T_hbm, w2T, sems.at[8])

    def wphi_copy():
        return pltpu.make_async_copy(wphi_hbm, wphi_scr, sems.at[9])

    def b1_copy():
        return pltpu.make_async_copy(b1_hbm, b1_scr, sems.at[10])

    def b2_copy():
        return pltpu.make_async_copy(b2_hbm, b2_scr, sems.at[11])

    def out_copy(t, k):
        lo, hi = OP[k]
        col = t * TS + lo
        if not isinstance(col, int):
            col = pl.multiple_of(col, 128)
        return pltpu.make_async_copy(o_scr.at[t, :, pl.ds(lo, hi - lo)], o_hbm.at[:, pl.ds(col, hi - lo)],
                                     osems.at[t * len(OP) + k])

    def layernorm(j):
        x = x_scr[:, j * 128:(j + 1) * 128].astype(f32)
        m = jnp.mean(x, axis=0, keepdims=True)
        xc = x - m
        var = jnp.mean(xc * xc, axis=0, keepdims=True)
        xn = xc * lax.rsqrt(var + EPS)
        rr = lax.broadcasted_iota(jnp.int32, (DP - D, 128), 0)
        xa = jnp.concatenate([xn, jnp.where(rr == 0, 1.0, 0.0)], axis=0).astype(bf16)
        xn_scr[:, j * 128:(j + 1) * 128] = _pk(xa)

    def phi_chunk(c):
        lo, hi = c * CW, (c + 1) * CW
        phi_scr[:, :, lo:hi] = _pk(_feature_map(_dot(_up(wk_scr[...]), _up(xn_scr[:, lo:hi]))))

    def v_piece(lo, hi):
        n = hi - lo
        vT = _dot(_up(wv_scr[...]), _up(xn_scr[:, lo:hi])).reshape(G, GR, n)
        ones = jnp.ones((G, 8, n), f32)
        va_scr[:, :, lo:hi] = _pk(jnp.concatenate([vT, ones], axis=1).astype(bf16))

    def kv_chunk(c):
        lo, hi = c * CW, (c + 1) * CW
        for g in range(G):
            new = _dot_nt(_up(va_scr[g, :, lo:hi]), _up(phi_scr[g, :, lo:hi]))
            if c == 0:
                kv_acc[g] = new
            else:
                kv_acc[g] += new

    def phase1():
        wphi_copy().start()
        wqkv_copy(0).start()
        x_copy(0).start()
        wqkv_copy(1).start()
        x_copy(1).start()
        zpad = jnp.zeros((D // 2, DP - D), u32)
        wk_scr[:, D:DP] = zpad
        wv_scr[:, D:DP] = zpad
        wq_scr[:, D:DP] = zpad
        a_scr[0:64, :] = jnp.zeros((64, DH), f32)
        a_scr[64 + D:128 + D, :] = jnp.zeros((64, DH), f32)
        wphi_copy().wait()
        p_scr[...] = wphi_scr[...].reshape(D, DH).astype(f32)
        for h in range(H):
            a_scr[64 + DH * h:64 + DH * (h + 1), :] = p_scr[pl.ds(h, DH, stride=H), :]
        bdt_k = _bdt_blocks(a_scr, D)
        wqkv_copy(0).wait()
        x_copy(2).start()
        wqkv_copy(2).start()
        b1_copy().start()
        b2_copy().start()
        w1_copy().start()
        wo_copy().start()
        w2_copy().start()
        wk_scr[:, 0:D] = _pk(_folded_weight(bdt_k, wqkv_scr, D))
        x_copy(0).wait()
        layernorm(0)
        layernorm(1)
        phi_chunk(0)
        wqkv_copy(1).wait()
        x_copy(1).wait()
        wv_scr[:, 0:D] = _pk(wqkv_scr[:, 2 * D:3 * D].T)
        for c in range(NC):
            if c == 2:
                x_copy(2).wait()
                wqkv_copy(2).wait()
            if c == W1_CHUNK:
                b1_copy().wait()
                b2_copy().wait()
                w1_copy().wait()
                wo_copy().wait()
            if c > 0:
                layernorm(2 * c + 1)
                phi_chunk(c)
            if c + 1 < NC:
                layernorm(2 * c + 2)
            v_piece(0 if c == 0 else c * CW + 128, min(c * CW + 384, S))
            if c > 0:
                kv_chunk(c - 1)
            if c == 2:
                wq_scr[:, 0:D] = _pk(_folded_weight(_bdt_blocks(a_scr, 0), wqkv_scr, 0))
            if c == W1_CHUNK:
                rr = lax.broadcasted_iota(jnp.int32, (DP - D, F), 0)
                w1raw[D:DP, :] = jnp.where(rr == 0, b1_scr[...].astype(f32).reshape(1, F), 0.0).astype(bf16)
                w1T[...] = _pk(w1raw[...].T)
                rr = lax.broadcasted_iota(jnp.int32, (DP - D, D), 0)
                woraw[D:DP, :] = jnp.where(rr == 0, b2_scr[...].astype(f32).reshape(1, D), 0.0).astype(bf16)
                woT[...] = _pk(woraw[...].T)
        kv_chunk(NC - 1)
        r = lax.broadcasted_iota(jnp.int32, (64, 2 * GR), 0)
        c = lax.broadcasted_iota(jnp.int32, (64, 2 * GR), 1)
        hr = jnp.where((r >= DH) & (r < GR) | (r >= 60), 1, 0)
        mask = hr == (c & 1)
        for g in range(G):
            kvT[g] = _pk(jnp.where(mask, kv_acc[g], 0.0).astype(bf16))
        w2_copy().wait()

    def tile2(t):
        col0 = pl.multiple_of(t * TS, TS)
        xa = _up(xn_scr[:, pl.ds(col0, TS)])
        phi = _feature_map(_dot(_up(wq_scr[...]), xa))
        sub = lax.broadcasted_iota(jnp.int32, (8, TS), 0)
        os = []
        for g in range(G):
            nd = _dot(_up(kvT[g]), phi[g])
            rd = 1.0 / (nd[GR:64] + 1e-6)
            rr = pltpu.roll(rd, 4, 0)
            r0 = jnp.where(sub < 4, rd, rr)
            r1 = jnp.where(sub < 4, rr, rd)
            scale = jnp.concatenate([r0, r0, r0, rd, r1, r1, r1], axis=0)
            os.append(nd[0:GR] * scale)
        rr = lax.broadcasted_iota(jnp.int32, (DP - D, TS), 0)
        os.append(jnp.where(rr == 0, 1.0, 0.0))
        oT = jnp.concatenate(os, axis=0).astype(bf16)
        hT = _dot(_up(w1T[...]), xa)
        c0 = 0.7978845608028654
        u = hT * (c0 + (c0 * 0.044715) * (hT * hT))
        gT = ((0.5 * hT) * (1.0 + jnp.tanh(u))).astype(bf16)
        woT_v = _up(woT[...])
        for k, (lo, hi) in enumerate(OP):
            outT = _dot(woT_v, oT[:, lo:hi]) + _dot(w2T[...], gT[:, lo:hi])
            xr = x_scr[:, pl.ds(pl.multiple_of(col0 + lo, 128), hi - lo)].astype(f32)
            o_scr[t, :, lo:hi] = (xr + outT).astype(bf16)
            out_copy(t, k).start()

    pl.when(i == 0)(phase1)

    @pl.when(i > 0)
    def _():
        for u in range(UN):
            tile2((i - 1) * UN + u)

    @pl.when(i == T // UN)
    def _():
        for t in range(T):
            for k in range(len(OP)):
                out_copy(t, k).wait()


@jax.jit
def pallas_parallel_sum__linear_kernel_hedgehog__dense_activation_gelu__prompt_kernel(
    A_x: jax.Array,
    A_wqkv: jax.Array,
    A_w_phi: jax.Array,
    A_wo: jax.Array,
    B_x: jax.Array,
    B_w1: jax.Array,
    B_b1: jax.Array,
    B_w2: jax.Array,
    B_b2: jax.Array,
):
    del B_x
    xT = A_x.reshape(S, D).T
    hbm = pl.BlockSpec(memory_space=pl.ANY)
    outT = pl.pallas_call(
        _kernel,
        grid=(T // UN + 1,),
        in_specs=[hbm] * 8,
        out_specs=hbm,
        out_shape=jax.ShapeDtypeStruct((D, S), bf16),
        scratch_shapes=[
            pltpu.VMEM((D, S), bf16),
            pltpu.VMEM((DP // 2, S), u32),
            pltpu.VMEM((D, 3 * D), bf16),
            pltpu.VMEM((D // 2, DP), u32),
            pltpu.VMEM((D // 2, DP), u32),
            pltpu.VMEM((D // 2, DP), u32),
            pltpu.VMEM((DP, F), bf16),
            pltpu.VMEM((F // 2, DP), u32),
            pltpu.VMEM((D, F), bf16),
            pltpu.VMEM((DP, D), bf16),
            pltpu.VMEM((D // 2, DP), u32),
            pltpu.VMEM((DH, H, DH), bf16),
            pltpu.VMEM((F,), bf16),
            pltpu.VMEM((D,), bf16),
            pltpu.VMEM((D, DH), f32),
            pltpu.VMEM((D + 128, DH), f32),
            pltpu.VMEM((G, 32, 2 * GR), u32),
            pltpu.VMEM((G, GR, S), u32),
            pltpu.VMEM((G, 32, S), u32),
            pltpu.VMEM((G, 64, 2 * GR), f32),
            pltpu.VMEM((T, D, TS), bf16),
            pltpu.SemaphoreType.DMA((12,)),
            pltpu.SemaphoreType.DMA((T * len(OP),)),
        ],
        compiler_params=pltpu.CompilerParams(
            dimension_semantics=("arbitrary",),
            vmem_limit_bytes=100 * 1024 * 1024,
        ),
    )(xT, A_wqkv, A_w_phi.transpose(1, 0, 2), B_b1, B_b2, A_wo, B_w1, B_w2.T)
    return outT.T.reshape(1, S, D)
```
